```python
import os as _os
_os.environ.setdefault("JAX_PLATFORMS", "cpu")
import jax
import jax.numpy as jnp

def _softmax(x, axis=-1):
    return jax.nn.softmax(x, axis=axis)
def _gelu(x):
    return jax.nn.gelu(x, approximate=True)
def _silu(x):
    return jax.nn.silu(x)
def _sigmoid(x):
    return jax.nn.sigmoid(x)
def _layernorm(x, axis=-1, eps=1e-5):
    m = jnp.mean(x, axis=axis, keepdims=True)
    v = jnp.var(x, axis=axis, keepdims=True)
    return (x - m) / jnp.sqrt(v + eps)
def _scatter_add(tgt, idx, src, axis=0):
    return tgt.at[idx].add(src)
def _segment_sum(src, seg, n):
    return jax.ops.segment_sum(src, seg, n)
class _Rng:
    def __init__(self, key):
        self._k = key
    def _next(self):
        self._k, sub = jax.random.split(self._k)
        return sub
    def normal(self, shape):
        return jax.random.normal(self._next(), shape, dtype=jnp.bfloat16)
    def randint(self, lo, hi, shape):
        return jax.random.randint(self._next(), shape, lo, hi, dtype=jnp.int32)
    def uniform(self, shape, lo=0.0, hi=1.0):
        return jax.random.uniform(self._next(), shape, jnp.bfloat16, lo, hi)
    def permutation(self, n):
        return jax.random.permutation(self._next(), n)


kernel_name = 'parallel_sum__sliding_local_dilated__glu_gated_geglu__prompt'

def setup_inputs():
    _rng = _Rng(jax.random.key(int.from_bytes(__import__("os").urandom(4), "little")))
    _w = (lambda a: (lambda t: t.astype(jnp.bfloat16) if jnp.issubdtype(t.dtype, jnp.floating) else t)(jnp.asarray(a)))
    def _A_setup():
        B, S, D = 1, 2048, 512
        return {
            "x": _w((lambda *s: _rng.normal(s) * 0.05)(B, S, D)),
            "wqkv": _w((lambda *s: _rng.normal(s) * 0.05)(D, 3 * D)),
            "wo": _w((lambda *s: _rng.normal(s) * 0.05)(D, D)),
        }
    _A_in = _A_setup()

    def _B_setup():
        B, S, Dm, Df = 1, 2048, 512, 1376
        return {
            "x": _w((lambda *s: _rng.normal(s) * 0.05)(B, S, Dm)),
            "w_gate": _w((lambda *s: _rng.normal(s) * 0.1)(Dm, Df) * (Dm ** -0.5)),
            "w_up": _w((lambda *s: _rng.normal(s) * 0.1)(Dm, Df) * (Dm ** -0.5)),
            "w_down": _w((lambda *s: _rng.normal(s) * 0.1)(Df, Dm) * (Df ** -0.5)),
        }
    _B_in = _B_setup()

    return {
        "A_x": _A_in["x"],
        "A_wqkv": _A_in["wqkv"],
        "A_wo": _A_in["wo"],
        "B_x": _B_in["x"],
        "B_w_gate": _B_in["w_gate"],
        "B_w_up": _B_in["w_up"],
        "B_w_down": _B_in["w_down"],
    }

def reference(A_x, A_wqkv, A_wo, B_x, B_w_gate, B_w_up, B_w_down):
    def _A_ref(x, wqkv, wo):
        B, S, D = x.shape
        H = 32; Dh = D // H
        W, dil = 8, 2
        qkv = (lambda x, *d: x.transpose(*d))((x @ wqkv).reshape(B, S, 3, H, Dh), 2, 0, 3, 1, 4)
        q, k, v = qkv[0], qkv[1], qkv[2]
        scale = Dh ** -0.5
        pos = jnp.arange(S)
        off = jnp.arange(W) * dil
        idx = pos[:, None] - off[None, :]
        mask = idx >= 0
        idx_c = jnp.where(mask, idx, 0).reshape(-1)
        kg = k[:, :, idx_c, :].reshape(B, H, S, W, Dh)
        vg = v[:, :, idx_c, :].reshape(B, H, S, W, Dh)
        logits = jnp.einsum("bhsd,bhswd->bhsw", q, kg) * scale
        logits = jnp.where(mask[None, None, :, :], logits, -1e9)
        attn = _softmax(logits, axis=-1)
        o = jnp.einsum("bhsw,bhswd->bhsd", attn, vg)
        return (lambda x, *d: x.transpose(*d))(o, 0, 2, 1, 3).reshape(B, S, D) @ wo

    def _B_ref(x, w_gate, w_up, w_down):
        g = jnp.einsum("bsd,df->bsf", x, w_gate)
        u = jnp.einsum("bsd,df->bsf", x, w_up)
        h = _gelu(g) * u
        return jnp.einsum("bsf,fd->bsd", h, w_down)

    x = A_x
    xn = _layernorm(x, axis=-1)
    return x + _A_ref(xn, A_wqkv, A_wo) + _B_ref(xn, B_w_gate, B_w_up, B_w_down)
```

```python
import functools

import jax
import jax.numpy as jnp
from jax import lax
import jax.experimental.pallas as pl
import jax.experimental.pallas.tpu as pltpu

_H = 32
_DH = 16
_W = 8
_DIL = 2
_HALO = 16
_EPS = 1e-5
_NEG = -1e9
_GELU_C = 0.7978845608028654


def _gelu_tanh(g):
    return 0.5 * g * (1.0 + jnp.tanh(_GELU_C * (g + 0.044715 * (g * g * g))))


def _kernel(x_ref, wqkv_hbm, wo_hbm, wg_hbm, wu_hbm, wd_hbm, o_ref,
            wqkv_raw, wo_raw, wo_f32, wqkv_p, wo_p, wg_s, wu_s, wd_s, kv_scr,
            sems, *, T, D):
    f32 = jnp.float32
    bf16 = jnp.bfloat16
    step = pl.program_id(0)

    def copies():
        cs = []
        for part in range(3):
            cs.append(pltpu.make_async_copy(
                wqkv_hbm.at[:, pl.ds(part * D, D)], wqkv_raw.at[part],
                sems.at[part]))
        cs.append(pltpu.make_async_copy(wo_hbm, wo_raw, sems.at[3]))
        cs.append(pltpu.make_async_copy(wg_hbm, wg_s, sems.at[4]))
        cs.append(pltpu.make_async_copy(wu_hbm, wu_s, sems.at[5]))
        cs.append(pltpu.make_async_copy(wd_hbm, wd_s, sems.at[6]))
        return cs

    def main(wait):
        x = x_ref[...].astype(f32)
        mu = jnp.mean(x, axis=-1, keepdims=True)
        xc = x - mu
        var = jnp.mean(xc * xc, axis=-1, keepdims=True)
        xn = (xc * lax.rsqrt(var + _EPS)).astype(bf16)

        qkv = jnp.dot(xn, wqkv_p[...], preferred_element_type=f32)
        q = qkv[:, 0:D] * (_DH ** -0.5)
        kv_scr[pl.ds(_HALO, T), :] = qkv[:, D:3 * D]

        row = step * T + lax.broadcasted_iota(jnp.int32, (T, 128), 0)
        logits = []
        for w in range(_W):
            k_w = kv_scr[pl.ds(_HALO - _DIL * w, T), pl.ds(0, D)]
            p = q * k_w
            l = (p[:, 0:128] + p[:, 128:256]) + (p[:, 256:384] + p[:, 384:512])
            l = l + pltpu.roll(l, 64, 1)
            l = l + pltpu.roll(l, 32, 1)
            if w > 0:
                l = jnp.where(row >= _DIL * w, l, _NEG)
            logits.append(l)
        m = logits[0]
        for w in range(1, _W):
            m = jnp.maximum(m, logits[w])
        es = [jnp.exp(l - m) for l in logits]
        den = es[0]
        for w in range(1, _W):
            den = den + es[w]
        r = 1.0 / den
        acc = [None] * 4
        for w in range(_W):
            a = es[w] * r
            v_w = kv_scr[pl.ds(_HALO - _DIL * w, T), pl.ds(D, D)]
            for j in range(4):
                t = a * v_w[:, j * 128:(j + 1) * 128]
                acc[j] = t if acc[j] is None else acc[j] + t
        o = jnp.concatenate(acc, axis=1).astype(bf16)
        kv_scr[pl.ds(0, _HALO), :] = kv_scr[pl.ds(T, _HALO), :]
        a_out = jnp.dot(o, wo_p[...], preferred_element_type=f32)

        wait(4)
        g = jnp.dot(xn, wg_s[...], preferred_element_type=f32)
        wait(5)
        u = jnp.dot(xn, wu_s[...], preferred_element_type=f32)
        h = (_gelu_tanh(g) * u).astype(bf16)
        wait(6)
        b_out = jnp.dot(h, wd_s[...], preferred_element_type=f32)

        o_ref[...] = (x + a_out + b_out).astype(o_ref.dtype)

    @pl.when(step == 0)
    def _():
        cs = copies()
        for c in cs:
            c.start()
        kv_scr[pl.ds(0, _HALO), :] = jnp.zeros((_HALO, 2 * D), f32)
        ci = lax.broadcasted_iota(jnp.int32, (D, D), 0)
        cj = lax.broadcasted_iota(jnp.int32, (D, D), 1)
        perm = jnp.where(cj == (ci % _DH) * _H + ci // _DH, 1.0, 0.0).astype(bf16)
        for part in range(3):
            cs[part].wait()
            wqkv_p[:, pl.ds(part * D, D)] = jnp.dot(
                wqkv_raw[part], perm, preferred_element_type=f32).astype(bf16)
        cs[3].wait()
        for j in range(D // 128):
            wo_f32[j] = wo_raw[:, pl.ds(j * 128, 128)].astype(f32)
        for d in range(_DH):
            for j in range(D // 128):
                wo_p[pl.ds(d * _H, _H), pl.ds(j * 128, 128)] = wo_f32[
                    j, pl.ds(d, _H, stride=_DH), :].astype(bf16)
        main(lambda i: cs[i].wait())

    @pl.when(step > 0)
    def _():
        main(lambda i: None)


@jax.jit
def pallas_parallel_sum__sliding_local_dilated__glu_gated_geglu__prompt_kernel(
    A_x: jax.Array,
    A_wqkv: jax.Array,
    A_wo: jax.Array,
    B_x: jax.Array,
    B_w_gate: jax.Array,
    B_w_up: jax.Array,
    B_w_down: jax.Array,
):
    B, S, D = A_x.shape
    DF = B_w_gate.shape[1]
    T = 256
    x2 = A_x.reshape(B * S, D)
    bf16 = jnp.bfloat16
    f32 = jnp.float32

    kernel = functools.partial(_kernel, T=T, D=D)
    out = pl.pallas_call(
        kernel,
        grid=(S // T,),
        in_specs=[
            pl.BlockSpec((T, D), lambda i: (i, 0)),
            pl.BlockSpec(memory_space=pl.ANY),
            pl.BlockSpec(memory_space=pl.ANY),
            pl.BlockSpec(memory_space=pl.ANY),
            pl.BlockSpec(memory_space=pl.ANY),
            pl.BlockSpec(memory_space=pl.ANY),
        ],
        out_specs=pl.BlockSpec((T, D), lambda i: (i, 0)),
        out_shape=jax.ShapeDtypeStruct((B * S, D), A_x.dtype),
        scratch_shapes=[
            pltpu.VMEM((3, D, D), bf16),
            pltpu.VMEM((D, D), bf16),
            pltpu.VMEM((D // 128, D, 128), f32),
            pltpu.VMEM((D, 3 * D), bf16),
            pltpu.VMEM((D, D), bf16),
            pltpu.VMEM((D, DF), bf16),
            pltpu.VMEM((D, DF), bf16),
            pltpu.VMEM((DF, D), bf16),
            pltpu.VMEM((T + _HALO, 2 * D), f32),
            pltpu.SemaphoreType.DMA((7,)),
        ],
        compiler_params=pltpu.CompilerParams(
            dimension_semantics=("arbitrary",),
            vmem_limit_bytes=64 * 1024 * 1024,
        ),
    )(x2, A_wqkv, A_wo, B_w_gate, B_w_up, B_w_down)
    return out.reshape(B, S, D)
```

```python
import functools

import jax
import jax.numpy as jnp
from jax import lax
import jax.experimental.pallas as pl
import jax.experimental.pallas.tpu as pltpu

_H = 32
_DH = 16
_W = 8
_DIL = 2
_HALO = 16
_EPS = 1e-5
_NEG = -1e9
_GELU_C = 0.7978845608028654


def _gelu_tanh(g):
    return 0.5 * g * (1.0 + jnp.tanh(_GELU_C * (g + 0.044715 * (g * g * g))))


def _kernel(x_ref, wqkv_hbm, wo_hbm, wg_hbm, wu_hbm, wd_hbm, o_ref,
            wqkv_raw, wo_raw, wo_f32, wqkv_p, wo_p, wg_s, wu_s, wd_s, kv_scr,
            sems, *, T, D):
    f32 = jnp.float32
    bf16 = jnp.bfloat16
    step = pl.program_id(0)

    def copies():
        cs = []
        for part in range(3):
            cs.append(pltpu.make_async_copy(
                wqkv_hbm.at[:, pl.ds(part * D, D)], wqkv_raw.at[part],
                sems.at[part]))
        cs.append(pltpu.make_async_copy(wo_hbm, wo_raw, sems.at[3]))
        cs.append(pltpu.make_async_copy(wg_hbm, wg_s, sems.at[4]))
        cs.append(pltpu.make_async_copy(wu_hbm, wu_s, sems.at[5]))
        cs.append(pltpu.make_async_copy(wd_hbm, wd_s, sems.at[6]))
        return cs

    def main(wait):
        x = x_ref[...].astype(f32)
        mu = jnp.mean(x, axis=-1, keepdims=True)
        xc = x - mu
        var = jnp.mean(xc * xc, axis=-1, keepdims=True)
        xn = (xc * lax.rsqrt(var + _EPS)).astype(bf16)

        qkv = jnp.dot(xn, wqkv_p[...], preferred_element_type=f32)
        q = qkv[:, 0:D] * (_DH ** -0.5)
        kv_scr[pl.ds(_HALO, T), :] = qkv[:, D:3 * D]

        row = step * T + lax.broadcasted_iota(jnp.int32, (T, 128), 0)
        logits = []
        for w in range(_W):
            k_w = kv_scr[pl.ds(_HALO - _DIL * w, T), pl.ds(0, D)]
            p = q * k_w
            l = (p[:, 0:128] + p[:, 128:256]) + (p[:, 256:384] + p[:, 384:512])
            l = l + pltpu.roll(l, 64, 1)
            l = l + pltpu.roll(l, 32, 1)
            if w > 0:
                l = jnp.where(row >= _DIL * w, l, _NEG)
            logits.append(l)
        m = logits[0]
        for w in range(1, _W):
            m = jnp.maximum(m, logits[w])
        es = [jnp.exp(l - m) for l in logits]
        den = es[0]
        for w in range(1, _W):
            den = den + es[w]
        r = 1.0 / den
        acc = [None] * 4
        for w in range(_W):
            a = es[w] * r
            v_w = kv_scr[pl.ds(_HALO - _DIL * w, T), pl.ds(D, D)]
            for j in range(4):
                t = a * v_w[:, j * 128:(j + 1) * 128]
                acc[j] = t if acc[j] is None else acc[j] + t
        o = jnp.concatenate(acc, axis=1).astype(bf16)
        kv_scr[pl.ds(0, _HALO), :] = kv_scr[pl.ds(T, _HALO), :]
        a_out = jnp.dot(o, wo_p[...], preferred_element_type=f32)

        wait(4)
        nt = (((1,), (1,)), ((), ()))
        g = lax.dot_general(xn, wg_s[...], nt, preferred_element_type=f32)
        wait(5)
        u = lax.dot_general(xn, wu_s[...], nt, preferred_element_type=f32)
        h = (_gelu_tanh(g) * u).astype(bf16)
        wait(6)
        b_out = jnp.dot(h, wd_s[...], preferred_element_type=f32)

        o_ref[...] = (x + a_out + b_out).astype(o_ref.dtype)

    @pl.when(step == 0)
    def _():
        cs = copies()
        for c in cs:
            c.start()
        kv_scr[pl.ds(0, _HALO), :] = jnp.zeros((_HALO, 2 * D), f32)
        ci = lax.broadcasted_iota(jnp.int32, (D, D), 0)
        cj = lax.broadcasted_iota(jnp.int32, (D, D), 1)
        perm = jnp.where(cj == (ci % _DH) * _H + ci // _DH, 1.0, 0.0).astype(bf16)
        for part in range(3):
            cs[part].wait()
            wqkv_p[:, pl.ds(part * D, D)] = jnp.dot(
                wqkv_raw[part], perm, preferred_element_type=f32).astype(bf16)
        cs[3].wait()
        for j in range(D // 128):
            wo_f32[j] = wo_raw[:, pl.ds(j * 128, 128)].astype(f32)
        for d in range(_DH):
            for j in range(D // 128):
                wo_p[pl.ds(d * _H, _H), pl.ds(j * 128, 128)] = wo_f32[
                    j, pl.ds(d, _H, stride=_DH), :].astype(bf16)
        main(lambda i: cs[i].wait())

    @pl.when(step > 0)
    def _():
        main(lambda i: None)


@jax.jit
def pallas_parallel_sum__sliding_local_dilated__glu_gated_geglu__prompt_kernel(
    A_x: jax.Array,
    A_wqkv: jax.Array,
    A_wo: jax.Array,
    B_x: jax.Array,
    B_w_gate: jax.Array,
    B_w_up: jax.Array,
    B_w_down: jax.Array,
):
    B, S, D = A_x.shape
    DF = B_w_gate.shape[1]
    T = 256
    x2 = A_x.reshape(B * S, D)
    bf16 = jnp.bfloat16
    f32 = jnp.float32

    kernel = functools.partial(_kernel, T=T, D=D)
    out = pl.pallas_call(
        kernel,
        grid=(S // T,),
        in_specs=[
            pl.BlockSpec((T, D), lambda i: (i, 0)),
            pl.BlockSpec(memory_space=pl.ANY),
            pl.BlockSpec(memory_space=pl.ANY),
            pl.BlockSpec(memory_space=pl.ANY),
            pl.BlockSpec(memory_space=pl.ANY),
            pl.BlockSpec(memory_space=pl.ANY),
        ],
        out_specs=pl.BlockSpec((T, D), lambda i: (i, 0)),
        out_shape=jax.ShapeDtypeStruct((B * S, D), A_x.dtype),
        scratch_shapes=[
            pltpu.VMEM((3, D, D), bf16),
            pltpu.VMEM((D, D), bf16),
            pltpu.VMEM((D // 128, D, 128), f32),
            pltpu.VMEM((D, 3 * D), bf16),
            pltpu.VMEM((D, D), bf16),
            pltpu.VMEM((DF, D), bf16),
            pltpu.VMEM((DF, D), bf16),
            pltpu.VMEM((DF, D), bf16),
            pltpu.VMEM((T + _HALO, 2 * D), f32),
            pltpu.SemaphoreType.DMA((7,)),
        ],
        compiler_params=pltpu.CompilerParams(
            dimension_semantics=("arbitrary",),
            vmem_limit_bytes=120 * 1024 * 1024,
        ),
    )(x2, A_wqkv, A_wo, B_w_gate.T, B_w_up.T, B_w_down)
    return out.reshape(B, S, D)
```

```python
import functools

import jax
import jax.numpy as jnp
from jax import lax
import jax.experimental.pallas as pl
import jax.experimental.pallas.tpu as pltpu

_H = 32
_DH = 16
_W = 8
_DIL = 2
_HALO = 16
_EPS = 1e-5
_NEG = -1e9
_GELU_C = 0.7978845608028654
_RC = 16
_PITCH = _DH + 1
_AH = 4


def _gelu_tanh(g):
    return 0.5 * g * (1.0 + jnp.tanh(_GELU_C * (g + 0.044715 * (g * g * g))))


def _kernel(x_hbm, wqkv_hbm, wo_hbm, wg_hbm, wu_hbm, wd_hbm,
            o_ref, x_scr, wqkv_raw, wo_raw, wo_f32, wqkv_p, wo_p, wg_s, wu_s,
            wd_s, kv_scr, q_scr, xn_scr, att_scr, wsems, xsems,
            *, T, D, NT):
    f32 = jnp.float32
    bf16 = jnp.bfloat16
    step = pl.program_id(0)
    NB = D // 128
    nt_dims = (((1,), (1,)), ((), ()))

    def x_copy(tile):
        return pltpu.make_async_copy(
            x_hbm.at[pl.ds(tile * T, T)], x_scr.at[tile], xsems.at[tile])

    def w_copies():
        cs = []
        for part in range(3):
            cs.append(pltpu.make_async_copy(
                wqkv_hbm.at[:, pl.ds(part * D, D)], wqkv_raw.at[part],
                wsems.at[part]))
        cs.append(pltpu.make_async_copy(wo_hbm, wo_raw, wsems.at[3]))
        cs.append(pltpu.make_async_copy(wg_hbm, wg_s, wsems.at[4]))
        cs.append(pltpu.make_async_copy(wu_hbm, wu_s, wsems.at[5]))
        cs.append(pltpu.make_async_copy(wd_hbm, wd_s, wsems.at[6]))
        return cs

    def layernorm(tile):
        x = x_scr[tile].astype(f32)
        mu = jnp.mean(x, axis=-1, keepdims=True)
        xc = x - mu
        var = jnp.mean(xc * xc, axis=-1, keepdims=True)
        xn_scr[tile] = (xc * lax.rsqrt(var + _EPS)).astype(bf16)

    def attention_chunk(r0, row0, z):
        qs = [q_scr[j, pl.ds(row0 + r0, _RC), :] for j in range(NB)]
        if z is not None:
            qs = [qj + z for qj in qs]
        logits = []
        for w in range(_W):
            base = row0 + (_HALO + r0 - _DIL * w)
            ps = [qs[j] * kv_scr[j, pl.ds(base, _RC), :] for j in range(NB)]
            l = (ps[0] + ps[1]) + (ps[2] + ps[3])
            l = l + pltpu.roll(l, 64, 1)
            l = l + pltpu.roll(l, 32, 1)
            if r0 < _DIL * w:
                row = row0 + r0 + lax.broadcasted_iota(jnp.int32, (_RC, 128), 0)
                l = jnp.where(row >= _DIL * w, l, _NEG)
            logits.append(l)
        m = logits[0]
        for w in range(1, _W):
            m = jnp.maximum(m, logits[w])
        es = [jnp.exp(l - m) for l in logits]
        den = es[0]
        for w in range(1, _W):
            den = den + es[w]
        r = 1.0 / den
        for j in range(NB):
            acc = None
            for w in range(_W):
                base = row0 + (_HALO + r0 - _DIL * w)
                t = es[w] * kv_scr[NB + j, pl.ds(base, _RC), :]
                acc = t if acc is None else acc + t
            att_scr[pl.ds(r0, _RC), pl.ds(j * 128, 128)] = (
                acc * r).astype(bf16)
        return jnp.where(r > 2.0, 1.0, 0.0)

    def qkv_matmul(tile, parts=(0, 1, 2)):
        lo, hi = parts[0] * D, (parts[-1] + 1) * D
        y = jnp.dot(xn_scr[tile], wqkv_p[:, pl.ds(lo, hi - lo)],
                    preferred_element_type=f32)
        row0 = pl.multiple_of(tile * T, T)
        for jj in range(parts[0] * NB, (parts[-1] + 1) * NB):
            blk = y[:, jj * 128 - lo:(jj + 1) * 128 - lo]
            if jj < NB:
                q_scr[jj, pl.ds(row0, T), :] = blk * (_DH ** -0.5)
            else:
                kv_scr[jj - NB, pl.ds(row0 + _HALO, T), :] = blk

    def permute_part(part):
        ri = lax.broadcasted_iota(jnp.int32, (128, 128), 0)
        li = lax.broadcasted_iota(jnp.int32, (128, 128), 1)
        dd = ri % _DH
        hl = ri // _DH
        st = []
        for j in range(NB):
            tgt = (dd % 4) * 32 + ((j + dd // 4) % 4) * 8 + hl
            p1 = jnp.where(li == tgt, 1.0, 0.0).astype(bf16)
            sj = jnp.dot(wqkv_raw[part, :, pl.ds(j * 128, 128)], p1,
                         preferred_element_type=f32).astype(bf16)
            st.append(pltpu.bitcast(sj, jnp.uint32))
        slot = (lax.broadcasted_iota(jnp.int32, (D // 2, 128), 1) % 32) // 8
        for jt in range(NB):
            out = None
            for j in range(NB - 1, -1, -1):
                shift = ((j - (j + jt) % 4) * 8) % 128
                rj = st[j] if shift == 0 else pltpu.roll(st[j], shift, 1)
                out = rj if out is None else jnp.where(slot == j, rj, out)
            wqkv_p[:, pl.ds(part * D + jt * 128, 128)] = pltpu.bitcast(out, bf16)

    def tile_out(tile):
        xn = xn_scr[tile]
        g = lax.dot_general(xn, wg_s[...], nt_dims, preferred_element_type=f32)
        z = None
        for c in range(T // _RC):
            z = attention_chunk(c * _RC, pl.multiple_of(tile * T, T), z)
        u = lax.dot_general(xn, wu_s[...], nt_dims, preferred_element_type=f32)
        h = (_gelu_tanh(g) * u).astype(bf16)
        b_out = jnp.dot(h, wd_s[...], preferred_element_type=f32)
        a_out = jnp.dot(att_scr[...], wo_p[...], preferred_element_type=f32)
        o_ref[...] = (x_scr[tile].astype(f32) + a_out + b_out
                      ).astype(o_ref.dtype)

    @pl.when(step == 0)
    def _():
        cs = w_copies()
        cs[0].start()
        x_copy(0).start()
        cs[1].start()
        x_copy(1).start()
        cs[2].start()
        for t in range(2, _AH):
            x_copy(t).start()
        for c in cs[3:]:
            c.start()
        for t in range(_AH, NT):
            x_copy(t).start()
        for j in range(2 * NB):
            kv_scr[j, pl.ds(0, _HALO), :] = jnp.zeros((_HALO, 128), f32)
        cs[0].wait()
        permute_part(0)
        x_copy(0).wait()
        cs[1].wait()
        layernorm(0)
        permute_part(1)
        qkv_matmul(0, (0,))
        for t in range(1, _AH):
            x_copy(t).wait()
        cs[2].wait()
        for t in range(1, _AH):
            layernorm(t)
        permute_part(2)
        qkv_matmul(0, (1,))
        for t in range(1, _AH):
            qkv_matmul(t, (0, 1))
        for t in range(_AH):
            qkv_matmul(t, (2,))
        cs[3].wait()
        for hh in range(_H):
            for j in range(NB):
                wo_f32[j, pl.ds(hh * _PITCH, _DH), :] = wo_raw[
                    pl.ds(hh * _DH, _DH), pl.ds(j * 128, 128)].astype(f32)
        for d in range(_DH):
            for j in range(NB):
                wo_p[pl.ds(d * _H, _H), pl.ds(j * 128, 128)] = wo_f32[
                    j, pl.ds(d, _H, stride=_PITCH), :].astype(bf16)
        for c in cs[4:]:
            c.wait()

    @pl.when(jnp.logical_and(step > 0, step + _AH - 1 < NT))
    def _():
        x_copy(step + _AH - 1).wait()
        tile_out(step - 1)
        layernorm(step + _AH - 1)
        qkv_matmul(step + _AH - 1)

    @pl.when(step + _AH - 1 >= NT)
    def _():
        tile_out(step - 1)


@jax.jit
def pallas_parallel_sum__sliding_local_dilated__glu_gated_geglu__prompt_kernel(
    A_x: jax.Array,
    A_wqkv: jax.Array,
    A_wo: jax.Array,
    B_x: jax.Array,
    B_w_gate: jax.Array,
    B_w_up: jax.Array,
    B_w_down: jax.Array,
):
    B, S, D = A_x.shape
    DF = B_w_gate.shape[1]
    T = 256
    NT = S // T
    x2 = A_x.reshape(B * S, D)
    bf16 = jnp.bfloat16
    f32 = jnp.float32

    kernel = functools.partial(_kernel, T=T, D=D, NT=NT)
    out = pl.pallas_call(
        kernel,
        grid=(NT + 1,),
        in_specs=[pl.BlockSpec(memory_space=pl.ANY)] * 6,
        out_specs=pl.BlockSpec((T, D), lambda s: (jnp.maximum(s - 1, 0), 0)),
        out_shape=jax.ShapeDtypeStruct((B * S, D), A_x.dtype),
        scratch_shapes=[
            pltpu.VMEM((NT, T, D), bf16),
            pltpu.VMEM((3, D, D), bf16),
            pltpu.VMEM((D, D), bf16),
            pltpu.VMEM((D // 128, _H * _PITCH, 128), f32),
            pltpu.VMEM((D, 3 * D), bf16),
            pltpu.VMEM((D, D), bf16),
            pltpu.VMEM((DF, D), bf16),
            pltpu.VMEM((DF, D), bf16),
            pltpu.VMEM((DF, D), bf16),
            pltpu.VMEM((2 * D // 128, S + _HALO, 128), f32),
            pltpu.VMEM((D // 128, S, 128), f32),
            pltpu.VMEM((NT, T, D), bf16),
            pltpu.VMEM((T, D), bf16),
            pltpu.SemaphoreType.DMA((7,)),
            pltpu.SemaphoreType.DMA((NT,)),
        ],
        compiler_params=pltpu.CompilerParams(
            dimension_semantics=("arbitrary",),
            vmem_limit_bytes=120 * 1024 * 1024,
        ),
    )(x2, A_wqkv, A_wo, B_w_gate.T, B_w_up.T, B_w_down)
    return out.reshape(B, S, D)
```

```python
import functools

import jax
import jax.numpy as jnp
from jax import lax
import jax.experimental.pallas as pl
import jax.experimental.pallas.tpu as pltpu

_H = 32
_DH = 16
_W = 8
_DIL = 2
_HALO = 16
_EPS = 1e-5
_NEG = -1e9
_GELU_C = 0.7978845608028654
_RC = 16
_PITCH = _DH + 1
_AH = 4


def _gelu_tanh(g):
    return 0.5 * g * (1.0 + jnp.tanh(_GELU_C * (g + 0.044715 * (g * g * g))))


def _kernel(x_hbm, wqkv_hbm, wo_hbm, wg_hbm, wu_hbm, wd_hbm,
            o_ref, x_scr, wqkv_raw, wo_raw, wo_f32, wqkv_p, wo_p, wg_s, wu_s,
            wd_s, kv_scr, q_scr, xn_scr, att_scr, wsems, xsems,
            *, T, D, NT):
    f32 = jnp.float32
    bf16 = jnp.bfloat16
    step = pl.program_id(0)
    NB = D // 128
    nt_dims = (((1,), (1,)), ((), ()))

    def x_copy(tile):
        return pltpu.make_async_copy(
            x_hbm.at[pl.ds(tile * T, T)], x_scr.at[tile], xsems.at[tile])

    def w_copies():
        cs = []
        for part in range(3):
            cs.append(pltpu.make_async_copy(
                wqkv_hbm.at[:, pl.ds(part * D, D)], wqkv_raw.at[part],
                wsems.at[part]))
        cs.append(pltpu.make_async_copy(wo_hbm, wo_raw, wsems.at[3]))
        cs.append(pltpu.make_async_copy(wg_hbm, wg_s, wsems.at[4]))
        cs.append(pltpu.make_async_copy(wu_hbm, wu_s, wsems.at[5]))
        cs.append(pltpu.make_async_copy(wd_hbm, wd_s, wsems.at[6]))
        return cs

    def layernorm(tile):
        x = x_scr[tile].astype(f32)
        mu = jnp.mean(x, axis=-1, keepdims=True)
        xc = x - mu
        var = jnp.mean(xc * xc, axis=-1, keepdims=True)
        xn_scr[tile] = (xc * lax.rsqrt(var + _EPS)).astype(bf16)

    def attention_chunk(r0, row0, z):
        qs = [q_scr[j, pl.ds(row0 + r0, _RC), :] for j in range(NB)]
        if z is not None:
            qs = [qj + z for qj in qs]
        logits = []
        for w in range(_W):
            base = row0 + (_HALO + r0 - _DIL * w)
            ps = [qs[j] * kv_scr[j, pl.ds(base, _RC), :] for j in range(NB)]
            l = (ps[0] + ps[1]) + (ps[2] + ps[3])
            l = l + pltpu.roll(l, 64, 1)
            l = l + pltpu.roll(l, 32, 1)
            if r0 < _DIL * w:
                row = row0 + r0 + lax.broadcasted_iota(jnp.int32, (_RC, 128), 0)
                l = jnp.where(row >= _DIL * w, l, _NEG)
            logits.append(l)
        m = logits[0]
        for w in range(1, _W):
            m = jnp.maximum(m, logits[w])
        es = [jnp.exp(l - m) for l in logits]
        den = es[0]
        for w in range(1, _W):
            den = den + es[w]
        r = 1.0 / den
        for j in range(NB):
            acc = None
            for w in range(_W):
                base = row0 + (_HALO + r0 - _DIL * w)
                t = es[w] * kv_scr[NB + j, pl.ds(base, _RC), :]
                acc = t if acc is None else acc + t
            att_scr[pl.ds(r0, _RC), pl.ds(j * 128, 128)] = (
                acc * r).astype(bf16)
        return jnp.where(r > 2.0, 1.0, 0.0)

    def qkv_matmul(tile, parts=(0, 1, 2)):
        lo, hi = parts[0] * D, (parts[-1] + 1) * D
        y = jnp.dot(xn_scr[tile], wqkv_p[:, pl.ds(lo, hi - lo)],
                    preferred_element_type=f32)
        row0 = pl.multiple_of(tile * T, T)
        for jj in range(parts[0] * NB, (parts[-1] + 1) * NB):
            blk = y[:, jj * 128 - lo:(jj + 1) * 128 - lo]
            if jj < NB:
                q_scr[jj, pl.ds(row0, T), :] = blk * (_DH ** -0.5)
            else:
                kv_scr[jj - NB, pl.ds(row0 + _HALO, T), :] = blk

    def permute_part(part):
        ri = lax.broadcasted_iota(jnp.int32, (128, 128), 0)
        li = lax.broadcasted_iota(jnp.int32, (128, 128), 1)
        dd = ri % _DH
        hl = ri // _DH
        st = []
        for j in range(NB):
            tgt = (dd % 4) * 32 + ((j + dd // 4) % 4) * 8 + hl
            p1 = jnp.where(li == tgt, 1.0, 0.0).astype(bf16)
            sj = jnp.dot(wqkv_raw[part, :, pl.ds(j * 128, 128)], p1,
                         preferred_element_type=f32).astype(bf16)
            st.append(pltpu.bitcast(sj, jnp.uint32))
        slot = (lax.broadcasted_iota(jnp.int32, (D // 2, 128), 1) % 32) // 8
        for jt in range(NB):
            out = None
            for j in range(NB - 1, -1, -1):
                shift = ((j - (j + jt) % 4) * 8) % 128
                rj = st[j] if shift == 0 else pltpu.roll(st[j], shift, 1)
                out = rj if out is None else jnp.where(slot == j, rj, out)
            wqkv_p[:, pl.ds(part * D + jt * 128, 128)] = pltpu.bitcast(out, bf16)

    def tile_out(tile):
        xn = xn_scr[tile]
        g = lax.dot_general(xn, wg_s[...], nt_dims, preferred_element_type=f32)
        z = None
        for c in range(T // _RC):
            z = attention_chunk(c * _RC, pl.multiple_of(tile * T, T), z)
        u = lax.dot_general(xn, wu_s[...], nt_dims, preferred_element_type=f32)
        h = (_gelu_tanh(g) * u).astype(bf16)
        b_out = jnp.dot(h, wd_s[...], preferred_element_type=f32)
        a_out = jnp.dot(att_scr[...], wo_p[...], preferred_element_type=f32)
        o_ref[...] = (x_scr[tile].astype(f32) + a_out + b_out
                      ).astype(o_ref.dtype)

    @pl.when(step == 0)
    def _():
        cs = w_copies()
        cs[0].start()
        x_copy(0).start()
        cs[1].start()
        x_copy(1).start()
        cs[2].start()
        for t in range(2, _AH):
            x_copy(t).start()
        for c in cs[3:]:
            c.start()
        for t in range(_AH, NT):
            x_copy(t).start()
        for j in range(2 * NB):
            kv_scr[j, pl.ds(0, _HALO), :] = jnp.zeros((_HALO, 128), f32)
        cs[0].wait()
        permute_part(0)
        x_copy(0).wait()
        cs[1].wait()
        layernorm(0)
        permute_part(1)
        qkv_matmul(0, (0,))
        x_copy(1).wait()
        cs[2].wait()
        layernorm(1)
        permute_part(2)
        qkv_matmul(0, (1,))
        qkv_matmul(1, (0, 1))
        qkv_matmul(0, (2,))
        for t in range(2, _AH):
            x_copy(t).wait()
        for t in range(2, _AH):
            layernorm(t)
        qkv_matmul(1, (2,))
        for t in range(2, _AH):
            qkv_matmul(t)
        cs[3].wait()
        for hh in range(_H):
            for j in range(NB):
                wo_f32[j, pl.ds(hh * _PITCH, _DH), :] = wo_raw[
                    pl.ds(hh * _DH, _DH), pl.ds(j * 128, 128)].astype(f32)
        for d in range(_DH):
            for j in range(NB):
                wo_p[pl.ds(d * _H, _H), pl.ds(j * 128, 128)] = wo_f32[
                    j, pl.ds(d, _H, stride=_PITCH), :].astype(bf16)
        for c in cs[4:]:
            c.wait()

    @pl.when(jnp.logical_and(step > 0, step + _AH - 1 < NT))
    def _():
        x_copy(step + _AH - 1).wait()
        tile_out(step - 1)
        layernorm(step + _AH - 1)
        qkv_matmul(step + _AH - 1)

    @pl.when(step + _AH - 1 >= NT)
    def _():
        tile_out(step - 1)


@jax.jit
def pallas_parallel_sum__sliding_local_dilated__glu_gated_geglu__prompt_kernel(
    A_x: jax.Array,
    A_wqkv: jax.Array,
    A_wo: jax.Array,
    B_x: jax.Array,
    B_w_gate: jax.Array,
    B_w_up: jax.Array,
    B_w_down: jax.Array,
):
    B, S, D = A_x.shape
    DF = B_w_gate.shape[1]
    T = 256
    NT = S // T
    x2 = A_x.reshape(B * S, D)
    bf16 = jnp.bfloat16
    f32 = jnp.float32

    kernel = functools.partial(_kernel, T=T, D=D, NT=NT)
    out = pl.pallas_call(
        kernel,
        grid=(NT + 1,),
        in_specs=[pl.BlockSpec(memory_space=pl.ANY)] * 6,
        out_specs=pl.BlockSpec((T, D), lambda s: (jnp.maximum(s - 1, 0), 0)),
        out_shape=jax.ShapeDtypeStruct((B * S, D), A_x.dtype),
        scratch_shapes=[
            pltpu.VMEM((NT, T, D), bf16),
            pltpu.VMEM((3, D, D), bf16),
            pltpu.VMEM((D, D), bf16),
            pltpu.VMEM((D // 128, _H * _PITCH, 128), f32),
            pltpu.VMEM((D, 3 * D), bf16),
            pltpu.VMEM((D, D), bf16),
            pltpu.VMEM((DF, D), bf16),
            pltpu.VMEM((DF, D), bf16),
            pltpu.VMEM((DF, D), bf16),
            pltpu.VMEM((2 * D // 128, S + _HALO, 128), f32),
            pltpu.VMEM((D // 128, S, 128), f32),
            pltpu.VMEM((NT, T, D), bf16),
            pltpu.VMEM((T, D), bf16),
            pltpu.SemaphoreType.DMA((7,)),
            pltpu.SemaphoreType.DMA((NT,)),
        ],
        compiler_params=pltpu.CompilerParams(
            dimension_semantics=("arbitrary",),
            vmem_limit_bytes=120 * 1024 * 1024,
        ),
    )(x2, A_wqkv, A_wo, B_w_gate.T, B_w_up.T, B_w_down)
    return out.reshape(B, S, D)
```
